```python
import os as _os
_os.environ.setdefault("JAX_PLATFORMS", "cpu")
import jax
import jax.numpy as jnp

def _softmax(x, axis=-1):
    return jax.nn.softmax(x, axis=axis)
def _gelu(x):
    return jax.nn.gelu(x, approximate=True)
def _silu(x):
    return jax.nn.silu(x)
def _sigmoid(x):
    return jax.nn.sigmoid(x)
def _layernorm(x, axis=-1, eps=1e-5):
    m = jnp.mean(x, axis=axis, keepdims=True)
    v = jnp.var(x, axis=axis, keepdims=True)
    return (x - m) / jnp.sqrt(v + eps)
def _scatter_add(tgt, idx, src, axis=0):
    return tgt.at[idx].add(src)
def _segment_sum(src, seg, n):
    return jax.ops.segment_sum(src, seg, n)
class _Rng:
    def __init__(self, key):
        self._k = key
    def _next(self):
        self._k, sub = jax.random.split(self._k)
        return sub
    def normal(self, shape):
        return jax.random.normal(self._next(), shape, dtype=jnp.bfloat16)
    def randint(self, lo, hi, shape):
        return jax.random.randint(self._next(), shape, lo, hi, dtype=jnp.int32)
    def uniform(self, shape, lo=0.0, hi=1.0):
        return jax.random.uniform(self._next(), shape, jnp.bfloat16, lo, hi)
    def permutation(self, n):
        return jax.random.permutation(self._next(), n)


kernel_name = 'concat_heads__mha_block_cached__gqa_block_cached__near_ridge'

def setup_inputs():
    _rng = _Rng(jax.random.key(int.from_bytes(__import__("os").urandom(4), "little")))
    _w = (lambda a: (lambda t: t.astype(jnp.bfloat16) if jnp.issubdtype(t.dtype, jnp.floating) else t)(jnp.asarray(a)))
    def _A_setup():
        B, Sq, D = 8, 128, 512
        H, Sk, Dh = 32, 1024, 128
        return {
            "x": _w((lambda *s: _rng.normal(s) * 0.8)(B, Sq, D)),
            "k_cache": _w((lambda *s: _rng.normal(s) * 0.8)(B, H, Sk, Dh)),
            "v_cache": _w((lambda *s: _rng.normal(s) * 0.05)(B, H, Sk, Dh)),
            "wq": _w((lambda *s: _rng.normal(s) * 0.8)(D, H * Dh) * (D ** -0.5)),
            "wo": _w((lambda *s: _rng.normal(s) * 0.05)(H * Dh, D) * ((H * Dh) ** -0.5)),
        }
    _A_in = _A_setup()

    def _B_setup():
        B, Sq, D = 8, 128, 512
        Hq, Hkv, Sk, Dh = 32, 32, 1024, 128
        assert Hq % Hkv == 0, (Hq, Hkv)
        return {
            "x": _w((lambda *s: _rng.normal(s) * 0.8)(B, Sq, D)),
            "k_cache": _w((lambda *s: _rng.normal(s) * 0.8)(B, Hkv, Sk, Dh)),
            "v_cache": _w((lambda *s: _rng.normal(s) * 0.05)(B, Hkv, Sk, Dh)),
            "wq": _w((lambda *s: _rng.normal(s) * 0.8)(D, Hq * Dh) * (D ** -0.5)),
            "wo": _w((lambda *s: _rng.normal(s) * 0.05)(Hq * Dh, D) * ((Hq * Dh) ** -0.5)),
        }
    _B_in = _B_setup()

    return {
        "A_x": _A_in["x"],
        "A_k_cache": _A_in["k_cache"],
        "A_v_cache": _A_in["v_cache"],
        "A_wq": _A_in["wq"],
        "A_wo": _A_in["wo"],
        "B_x": _B_in["x"],
        "B_k_cache": _B_in["k_cache"],
        "B_v_cache": _B_in["v_cache"],
        "B_wq": _B_in["wq"],
        "B_wo": _B_in["wo"],
    }

def reference(A_x, A_k_cache, A_v_cache, A_wq, A_wo, B_x, B_k_cache, B_v_cache, B_wq, B_wo):
    def _A_ref(x, k_cache, v_cache, wq, wo):
        B, Sq, D = x.shape
        H, Dh = 32, 128
        q = (lambda x, *d: x.transpose(*d))((x @ wq).reshape(B, Sq, H, Dh), 0, 2, 1, 3)
        scores = jnp.einsum("bhqd,bhkd->bhqk", q, k_cache) * (Dh ** -0.5)
        p = _softmax(scores, axis=-1)
        o = jnp.einsum("bhqk,bhkd->bhqd", p, v_cache)
        return (lambda x, *d: x.transpose(*d))(o, 0, 2, 1, 3).reshape(B, Sq, H * Dh) @ wo

    def _B_ref(x, k_cache, v_cache, wq, wo):
        B, Sq, D = x.shape
        Hq, Dh = 32, 128
        Hkv = k_cache.shape[1]
        rep = Hq // Hkv
        q = (lambda x, *d: x.transpose(*d))((x @ wq).reshape(B, Sq, Hq, Dh), 0, 2, 1, 3)
        k = jnp.repeat(k_cache, rep, axis=1)
        v = jnp.repeat(v_cache, rep, axis=1)
        scores = jnp.einsum("bhqd,bhkd->bhqk", q, k) * (Dh ** -0.5)
        p = _softmax(scores, axis=-1)
        o = jnp.einsum("bhqk,bhkd->bhqd", p, v)
        return (lambda x, *d: x.transpose(*d))(o, 0, 2, 1, 3).reshape(B, Sq, Hq * Dh) @ wo

    a = _A_ref(A_x, A_k_cache, A_v_cache, A_wq, A_wo)
    b = _B_ref(B_x, B_k_cache, B_v_cache, B_wq, B_wo)
    return jnp.concatenate([a, b], axis=-1)
```

```python
import functools
import jax
import jax.numpy as jnp
import numpy as np
import jax.experimental.pallas as pl
import jax.experimental.pallas.tpu as pltpu

HB = 4
_C = float((128 ** -0.5) * 1.4426950408889634)

def _kern(ax, ak, av, awq, awo, bx, bk, bv, bwq, bwo, o_ref, acc):
    g = pl.program_id(1)
    W = HB * 128

    @pl.when(g == 0)
    def _():
        acc[...] = jnp.zeros_like(acc)

    off = pl.multiple_of(g * W, W)
    sides = ((ax, ak, av, awq, awo), (bx, bk, bv, bwq, bwo))
    def proj(sd):
        x, k, v, wq, wo = sides[sd]
        q = jnp.dot(x[0], wq[:, pl.ds(off, W)], preferred_element_type=jnp.float32)
        return (q * _C).astype(jnp.bfloat16)
    def qk(q, sd, h):
        return jax.lax.dot_general(q[:, h*128:(h+1)*128], sides[sd][1][0, h], (((1,), (1,)), ((), ())),
                                    preferred_element_type=jnp.float32)
    def pv(s, sd, h):
        m = jnp.max(s, axis=1, keepdims=True)
        p = jnp.exp2(s - m)
        l = jnp.sum(p, axis=1, keepdims=True)
        o = jnp.dot(p.astype(jnp.bfloat16), sides[sd][2][0, h], preferred_element_type=jnp.float32)
        return (o * (1.0 / l)).astype(jnp.bfloat16)
    def oproj(os_, sd):
        oc = jnp.concatenate(os_, axis=1)
        acc[:, sd*512:(sd+1)*512] += jnp.dot(oc, sides[sd][4][pl.ds(off, W), :], preferred_element_type=jnp.float32)
    items = [(sd, h) for sd in range(2) for h in range(HB)]
    q = [proj(0), None]
    S = {}
    O = [[], []]
    S[0] = qk(q[0], 0, 0)
    q[1] = proj(1)
    for i, (sd, h) in enumerate(items):
        if i + 1 < len(items):
            sd2, h2 = items[i+1]
            S[i+1] = qk(q[sd2], sd2, h2)
        if i == len(items) - 1:
            oproj(O[0], 0)
        O[sd].append(pv(S.pop(i), sd, h))
    oproj(O[1], 1)

    @pl.when(g == pl.num_programs(1) - 1)
    def _():
        o_ref[0] = acc[...].astype(o_ref.dtype)


@jax.jit
def pallas_concat_heads__mha_block_cached__gqa_block_cached__near_ridge_kernel(
        A_x, A_k_cache, A_v_cache, A_wq, A_wo, B_x, B_k_cache, B_v_cache, B_wq, B_wo):
    B, Sq, D = A_x.shape
    H, Sk, Dh = A_k_cache.shape[1:]
    xs = pl.BlockSpec((1, Sq, D), lambda b, g: (b, 0, 0))
    ks = pl.BlockSpec((1, HB, Sk, Dh), lambda b, g: (b, g, 0, 0))
    wqs = pl.BlockSpec((D, H * Dh), lambda b, g: (0, 0), pipeline_mode=pl.Buffered(1))
    wos = pl.BlockSpec((H * Dh, D), lambda b, g: (0, 0), pipeline_mode=pl.Buffered(1))
    return pl.pallas_call(
        _kern,
        grid=(B, H // HB),
        in_specs=[xs, ks, ks, wqs, wos] * 2,
        out_specs=pl.BlockSpec((1, Sq, 2 * D), lambda b, g: (b, 0, 0)),
        out_shape=jax.ShapeDtypeStruct((B, Sq, 2 * D), A_x.dtype),
        scratch_shapes=[pltpu.VMEM((Sq, 2 * D), jnp.float32)],
        compiler_params=pltpu.CompilerParams(
            dimension_semantics=("arbitrary", "arbitrary"),
            vmem_limit_bytes=100 * 1024 * 1024),
    )(A_x, A_k_cache, A_v_cache, A_wq, A_wo, B_x, B_k_cache, B_v_cache, B_wq, B_wo)
```

```python
import jax
import jax.numpy as jnp
import jax.experimental.pallas as pl
import jax.experimental.pallas.tpu as pltpu

HB = 2
NB = 3
_C = float((128 ** -0.5) * 1.4426950408889634)
B, SQ, D, H, SK, DH = 8, 128, 512, 32, 1024, 128
G = H // HB
T = B * G
W = HB * DH


def _kern(ax, ak, av, awq, awo, bx, bk, bv, bwq, bwo, o_hbm,
          xb, wqb, wob, kb, vb, acc, ob, xsem, wsem, kvsem, osem):
    X, K, V, WQ, WO = (ax, bx), (ak, bk), (av, bv), (awq, bwq), (awo, bwo)

    def x_cp(sd):
        return pltpu.make_async_copy(X[sd], xb.at[sd], xsem.at[sd])

    def wq_cp(sd, g):
        c = pl.ds(pl.multiple_of(g * W, W), W)
        return pltpu.make_async_copy(WQ[sd].at[:, c], wqb.at[sd, :, c], wsem.at[0, sd, g])

    def wo_cp(sd, g):
        c = pl.ds(pl.multiple_of(g * W, W), W)
        return pltpu.make_async_copy(WO[sd].at[c, :], wob.at[sd, c, :], wsem.at[1, sd, g])

    def k_cp(sd, t):
        s = t % NB
        return pltpu.make_async_copy(K[sd].at[pl.ds(t * HB, HB)], kb.at[s, sd], kvsem.at[0, s, sd])

    def v_cp(sd, t):
        s = t % NB
        return pltpu.make_async_copy(V[sd].at[pl.ds(t * HB, HB)], vb.at[s, sd], kvsem.at[1, s, sd])

    def o_cp(b):
        return pltpu.make_async_copy(ob.at[b % 2], o_hbm.at[b], osem.at[b % 2])

    for sd in range(2):
        x_cp(sd).start()
        wq_cp(sd, 0).start()
        k_cp(sd, 0).start()
    for sd in range(2):
        v_cp(sd, 0).start()
        wo_cp(sd, 0).start()
    for t in range(1, NB - 1):
        for sd in range(2):
            k_cp(sd, t).start()
        for sd in range(2):
            v_cp(sd, t).start()
    for sd in range(2):
        x_cp(sd).wait()

    def step(t, carry):
        b = t // G
        g = t % G

        @pl.when(t + NB - 1 < T)
        def _():
            for sd in range(2):
                k_cp(sd, t + NB - 1).start()
            for sd in range(2):
                v_cp(sd, t + NB - 1).start()

        @pl.when(t + 1 < G)
        def _():
            for sd in range(2):
                wq_cp(sd, t + 1).start()
                wo_cp(sd, t + 1).start()

        @pl.when(t < G)
        def _():
            for sd in range(2):
                wq_cp(sd, t).wait()
                wo_cp(sd, t).wait()

        @pl.when(g == 0)
        def _():
            acc[...] = jnp.zeros_like(acc)

        for sd in range(2):
            k_cp(sd, t).wait()
            v_cp(sd, t).wait()

        slot = t % NB
        off = pl.multiple_of(g * W, W)

        def proj(sd):
            q = jnp.dot(xb[sd, b], wqb[sd, :, pl.ds(off, W)], preferred_element_type=jnp.float32)
            return (q * _C).astype(jnp.bfloat16)

        def qk(q, sd, h):
            return jax.lax.dot_general(q[:, h*DH:(h+1)*DH], kb[slot, sd, h], (((1,), (1,)), ((), ())),
                                       preferred_element_type=jnp.float32)

        def pv(s, sd, h):
            m = jnp.max(s, axis=1, keepdims=True)
            p = jnp.exp2(s - m)
            l = jnp.sum(p, axis=1, keepdims=True)
            o = jnp.dot(p.astype(jnp.bfloat16), vb[slot, sd, h], preferred_element_type=jnp.float32)
            return (o * (1.0 / l)).astype(jnp.bfloat16)

        def oproj(os_, sd):
            oc = jnp.concatenate(os_, axis=1)
            acc[:, sd*D:(sd+1)*D] += jnp.dot(oc, wob[sd, pl.ds(off, W), :], preferred_element_type=jnp.float32)

        items = [(sd, h) for sd in range(2) for h in range(HB)]
        q = [proj(0), None]
        S = {}
        O = [[], []]
        S[0] = qk(q[0], 0, 0)
        q[1] = proj(1)
        for i, (sd, h) in enumerate(items):
            if i + 1 < len(items):
                sd2, h2 = items[i+1]
                S[i+1] = qk(q[sd2], sd2, h2)
            if i == len(items) - 1:
                oproj(O[0], 0)
            O[sd].append(pv(S.pop(i), sd, h))
        oproj(O[1], 1)

        @pl.when(g == G - 1)
        def _():
            @pl.when(b >= 2)
            def _():
                o_cp(b - 2).wait()
            ob[b % 2] = acc[...].astype(ob.dtype)
            o_cp(b).start()
        return carry

    jax.lax.fori_loop(0, T, step, 0)
    o_cp(B - 2).wait()
    o_cp(B - 1).wait()


@jax.jit
def pallas_concat_heads__mha_block_cached__gqa_block_cached__near_ridge_kernel(
        A_x, A_k_cache, A_v_cache, A_wq, A_wo, B_x, B_k_cache, B_v_cache, B_wq, B_wo):
    r = lambda a: a.reshape(B * H, SK, DH)
    bf = jnp.bfloat16
    return pl.pallas_call(
        _kern,
        in_specs=[pl.BlockSpec(memory_space=pl.ANY)] * 10,
        out_specs=pl.BlockSpec(memory_space=pl.ANY),
        out_shape=jax.ShapeDtypeStruct((B, SQ, 2 * D), A_x.dtype),
        scratch_shapes=[
            pltpu.VMEM((2, B, SQ, D), bf), pltpu.VMEM((2, D, H * DH), bf), pltpu.VMEM((2, H * DH, D), bf),
            pltpu.VMEM((NB, 2, HB, SK, DH), bf), pltpu.VMEM((NB, 2, HB, SK, DH), bf),
            pltpu.VMEM((SQ, 2 * D), jnp.float32), pltpu.VMEM((2, SQ, 2 * D), bf),
            pltpu.SemaphoreType.DMA((2,)), pltpu.SemaphoreType.DMA((2, 2, G)),
            pltpu.SemaphoreType.DMA((2, NB, 2)), pltpu.SemaphoreType.DMA((2,)),
        ],
        compiler_params=pltpu.CompilerParams(vmem_limit_bytes=100 * 1024 * 1024),
    )(A_x, r(A_k_cache), r(A_v_cache), A_wq, A_wo, B_x, r(B_k_cache), r(B_v_cache), B_wq, B_wo)
```
